```python
import os as _os
_os.environ.setdefault("JAX_PLATFORMS", "cpu")
import jax
import jax.numpy as jnp

def _softmax(x, axis=-1):
    return jax.nn.softmax(x, axis=axis)
def _gelu(x):
    return jax.nn.gelu(x, approximate=True)
def _silu(x):
    return jax.nn.silu(x)
def _sigmoid(x):
    return jax.nn.sigmoid(x)
def _layernorm(x, axis=-1, eps=1e-5):
    m = jnp.mean(x, axis=axis, keepdims=True)
    v = jnp.var(x, axis=axis, keepdims=True)
    return (x - m) / jnp.sqrt(v + eps)
def _scatter_add(tgt, idx, src, axis=0):
    return tgt.at[idx].add(src)
def _segment_sum(src, seg, n):
    return jax.ops.segment_sum(src, seg, n)
class _Rng:
    def __init__(self, key):
        self._k = key
    def _next(self):
        self._k, sub = jax.random.split(self._k)
        return sub
    def normal(self, shape):
        return jax.random.normal(self._next(), shape, dtype=jnp.bfloat16)
    def randint(self, lo, hi, shape):
        return jax.random.randint(self._next(), shape, lo, hi, dtype=jnp.int32)
    def uniform(self, shape, lo=0.0, hi=1.0):
        return jax.random.uniform(self._next(), shape, jnp.bfloat16, lo, hi)
    def permutation(self, n):
        return jax.random.permutation(self._next(), n)


kernel_name = 'standalone__seq2seq_rnn_t_joint__speech'

def setup_inputs():
    _rng = _Rng(jax.random.key(int.from_bytes(__import__("os").urandom(4), "little")))
    _w = (lambda a: (lambda t: t.astype(jnp.bfloat16) if jnp.issubdtype(t.dtype, jnp.floating) else t)(jnp.asarray(a)))
    B, T, D, K = 2, 1000, 512, 31
    U = 8
    sc = (1.0 / (K * D)) ** 0.5
    sd = (1.0 / D) ** 0.5
    return {
        "x": _w((lambda *s: _rng.normal(s) * 0.4)(B, T, D) * 0.5),
        "w1": _w((lambda *s: _rng.normal(s) * 1.6)(K, D, D) * sc),
        "w2": _w((lambda *s: _rng.normal(s) * 1.6)(K, D, D) * sc),
        "g": _w((lambda *s: _rng.normal(s) * 1.6)(B, U, D) * 0.5),
        "w_f": _w((lambda *s: _rng.normal(s) * 1.6)(D, D) * sd),
        "w_g": _w((lambda *s: _rng.normal(s) * 1.6)(D, D) * sd),
        "w_o": _w((lambda *s: _rng.normal(s) * 1.6)(D, D) * sd),
    }

def reference(x, w1, w2, g, w_f, w_g, w_o):
    B, T, D = x.shape
    K = w1.shape[0]
    pad = K // 2
    xp = jnp.pad(x, ((0,0),(pad,pad),(0,0)))
    h = jnp.zeros_like(x)
    for i in range(K):
        h = h + jnp.einsum("btc,cd->btd", xp[:, i:i+T, :], w1[i])
    h = _gelu(h)[:, ::2, :]
    T1 = h.shape[1]
    hp = jnp.pad(h, ((0,0),(pad,pad),(0,0)))
    f = jnp.zeros_like(h)
    for i in range(K):
        f = f + jnp.einsum("btc,cd->btd", hp[:, i:i+T1, :], w2[i])
    f = _gelu(f)[:, ::2, :]
    fe = jnp.einsum("btd,de->bte", f, w_f)
    ge = jnp.einsum("bud,de->bue", g, w_g)
    j = jnp.tanh(fe[:, :, None, :] + ge[:, None, :, :])
    return jnp.einsum("btud,dv->btuv", j, w_o)
```

```python
import numpy as np
import jax
import jax.numpy as jnp
import jax.experimental.pallas as pl
import jax.experimental.pallas.tpu as pltpu

B, T, D, K, U = 2, 1000, 512, 31, 8
T1, T2 = 500, 250
NCH = 8
P1, P2 = 64, 32
SL = 16
NT = D // 128
NJ = 27
F32, BF16, U32 = jnp.float32, jnp.bfloat16, jnp.uint32
HI = np.uint32(0xFFFF0000)


def _data_tree(d):
    m = (len(d) + 1) // 2
    if m == 1:
        yield d[0]
        return
    h = m // 2
    n = 2 * h - 1
    lo, mid, hi = d[0:n], d[h:h + n], d[2 * h:2 * h + n]
    yield from _data_tree([_sub2(x, y) for x, y in zip(lo, mid)])
    yield from _data_tree(mid)
    yield from _data_tree([_sub2(x, y) for x, y in zip(hi, mid)])


def _nadd(a, b):
    if a is None:
        return b
    if b is None:
        return a
    return (a, b)


def _node_tree(g):
    if len(g) == 1:
        return g
    h = len(g) // 2
    lo, hi = g[:h], g[h:]
    return _node_tree(lo) + _node_tree([_nadd(a, b) for a, b in zip(lo, hi)]) + _node_tree(hi)


def _cost(n):
    if not isinstance(n, tuple):
        return 0
    return 3 + 2 * sum(isinstance(c, int) for c in n)


def _order(nodes):
    done, out, heavy = set(), [], True
    while len(out) < len(nodes):
        rdy = [j for j, n in enumerate(nodes) if j not in out and
               (not isinstance(n, tuple) or all(isinstance(c, int) or c in done for c in n))]
        j = (max if heavy else min)(rdy, key=lambda j: (_cost(nodes[j]), -j if heavy else j))
        out.append(j)
        done.add(nodes[j])
        heavy = not heavy
    return out


def _out_tree(ms):
    if len(ms) == 1:
        return ms
    n = len(ms) // 3
    y0, y1, y2 = _out_tree(ms[:n]), _out_tree(ms[n:2 * n]), _out_tree(ms[2 * n:])
    return [p + q for p, q in zip(y0, y1)] + [p + q for p, q in zip(y1, y2)]


def _gelu(x):
    c = np.float32(np.sqrt(2 / np.pi))
    hx = 0.5 * x
    return hx + hx * jnp.tanh(x * (c + np.float32(0.044715 * np.sqrt(2 / np.pi)) * (x * x)))


XP = 84


def _pk(a, b):
    return pltpu.bitcast(pltpu.pack_elementwise([a, b], packed_dtype=BF16), U32)


def _sub2(x, y):
    return (x[0] - y[0], x[1] - y[1])


def _chain(tasks):
    for t in tasks:
        yield from t()


def _merge(main, n, *others):
    its = [(_chain(o), len(o) * c) for o, c in others]
    pos = [0] * len(its)
    for i, _ in enumerate(_chain(main)):
        for k, (it, tot) in enumerate(its):
            while pos[k] < ((i + 1) * tot) // n:
                next(it)
                pos[k] += 1
    for it, _ in its:
        for _ in it:
            pass


def _run(tasks):
    for _ in _chain(tasks):
        pass


PAIR, FL, SP, MW, FP = 1, 1, (0, 6, 12), 1, 4


def make():
    def kernel(x_hbm, w1_hbm, w2_hbm, g_hbm, wf_hbm, wg_hbm, wo_hbm, o_hbm,
               xb, wb, cf, gb, wfb, wgb, wob, d1, a1, hb, d2, a2, fb, feb, ob,
               sem_x, sem_w, sem_m, sem_o, sem_z, sem_f):
        lanes = lambda n: pl.ds(n * 128 if isinstance(n, int) else pl.multiple_of(n * 128, 128), 128)
        wv = wb.bitcast(BF16)
        zs, zl = pl.semaphore_read(sem_z.at[0]), pl.semaphore_read(sem_z.at[1])

        def wcopy(cv, nt, half):
            src = (w1_hbm, w2_hbm)[cv]
            n = 16 if half == 0 else 15
            return pltpu.make_async_copy(src.at[pl.ds(16 * half, n), :, lanes(nt)],
                                         wv.at[cv, nt, pl.ds(16 * half, n)],
                                         sem_w.at[(cv * NT + nt) * 2 + half])

        xv = xb.bitcast(BF16)
        def xcopy(b, lt, n):
            lo, hi = max(0, 2 * P1 * n - 16), min(T, 2 * P1 * n + 144)
            return pltpu.make_async_copy(
                x_hbm.at[b, pl.ds(lo, hi - lo), lanes(lt)],
                xv.at[n % 2, lt, pl.ds(2 * XP * (4 * b + n // 2) + lo - (2 * P1 * n - 16), hi - lo), :],
                sem_x.at[lt])
        small = [pltpu.make_async_copy(s, d, sem_m.at[i]) for i, (s, d) in
                 enumerate([(g_hbm, gb), (wf_hbm, wfb), (wg_hbm, wgb), (wo_hbm, wob)])]

        def taps_of(ks, ph):
            t = lambda k: 2 * k + ph if 2 * k + ph < K else None
            return [t(kk[0]) if len(kk) == 1 else _nadd(t(kk[0]), t(kk[1])) for kk in ks]
        def prods(cv, part):
            if cv == 0 and part == 1:
                ks = [[k, k + 8] for k in range(8)]
            else:
                ks = [[k + (4 * part if cv == 0 else 8 * part)] for k in range(8)]
            return [_node_tree(taps_of(ks, ph)) for ph in range(2)]

        first = [pltpu.make_async_copy(w1_hbm.at[pl.ds(FP * i, FP), :, lanes(0)],
                                       wv.at[0, 0, pl.ds(FP * i, FP)], sem_f.at[i]) for i in range(16 // FP)]

        def dot_tasks(cv, nt, part, fine=False):
            u = dict(prod=prods(cv, part))
            seen = set()
            def raw(t):
                if fine and t // FP not in seen:
                    seen.add(t // FP)
                    first[t // FP].wait()
                    if len(seen) == 8 // FP:
                        wcopy(0, 0, 1).start()
                return wb[cv, nt, t]
            slots = []
            for ph in range(2):
                kids = []
                for n in u["prod"][ph]:
                    if isinstance(n, tuple):
                        kids += [c for c in n if isinstance(c, tuple) and c not in kids]
                slots.append({c: i for i, c in enumerate(kids)})
            def weight(ph, n):
                if isinstance(n, int):
                    return raw(n)
                vs = []
                for c in n:
                    if isinstance(c, int):
                        w = raw(c)
                        vs.append((pltpu.bitcast(w << 16, F32), pltpu.bitcast(w & HI, F32)))
                    else:
                        vs.append((cf[ph][slots[ph][c]][zl], cf[ph][slots[ph][c]][zl + 1]))
                lo, hi = vs[0][0] + vs[1][0], vs[0][1] + vs[1][1]
                if n in slots[ph]:
                    cf[ph][slots[ph][n]][zs] = lo
                    cf[ph][slots[ph][n]][zs + 1] = hi
                return _pk(lo, hi)
            def task(js):
                def run():
                    acc = {j: a2[nt % 2, zl, j] if cv == 1 and part == 1 else None for j in js}
                    for ph in range(2):
                        for j in js:
                            n = u["prod"][ph][j]
                            if n is not None:
                                d = d1[part, ph + zl, j] if cv == 0 else d2[ph + zl, j, pl.ds(part * 8, 32), :]
                                r = jnp.dot(pltpu.bitcast(d, BF16), pltpu.bitcast(weight(ph, n), BF16),
                                            preferred_element_type=F32)
                                acc[j] = r if acc[j] is None else acc[j] + r
                            yield
                    for j in js:
                        (a1, a2)[cv][nt % 2, part + zs, j] = acc[j]
                return run
            o = _order(u["prod"][0])
            return [task(o[i:i + PAIR]) for i in range(0, NJ, PAIR)]

        def d1_tasks(part):
            o0, o1 = ((0, 8), (8, None), (16, 8))[part]
            def task(lt, s, ph):
                def run():
                    def val(q):
                        ws = [xb[e, lt, pl.ds(q + ph, 8, stride=XP), :] for e in range(2)]
                        return tuple(pltpu.bitcast(w & HI if ph == 0 else w << 16, F32) for w in ws)
                    if o1 is None:
                        d = [val(16 * s + o0 + r) for r in range(15)]
                    else:
                        c = {}
                        def cv(q):
                            if q not in c:
                                c[q] = val(q)
                            return c[q]
                        d = [_sub2(cv(16 * s + o0 + r), cv(16 * s + o1 + r)) for r in range(15)]
                    for j, v in enumerate(_data_tree(d)):
                        d1[part, ph + zs, j, pl.ds(s * 8, 8), lanes(lt)] = _pk(*v)
                        yield
                return run
            return [task(lt, s, ph) for lt in range(NT) for s in range(4) for ph in range(2)]

        sub = jax.lax.broadcasted_iota(jnp.int32, (NCH, 128), 0)

        sub4 = jax.lax.broadcasted_iota(jnp.int32, (8, 128), 0) % 4

        def post1_tasks(nt):
            def gel(s, b):
                def run():
                    rows = pl.ds(s * SL + b * NCH, NCH)
                    tree = lambda part: _out_tree([a1[nt % 2, part + zl, j, rows, :] for j in range(NJ)])
                    yb = tree(1)
                    yield from range(5)
                    for half in range(2):
                        ya = tree(2 * half)
                        yield from range(3)
                        for o in range(8):
                            p = 16 * s + 8 * half + o
                            h = _gelu(ya[o] + yb[o])
                            if p >= T1 - (NCH - 1) * P1:
                                h = jnp.where(sub == NCH - 1, 0.0, h)
                            hb[zs, pl.ds(p * SL + b * NCH, NCH), :] = h
                            yield
                return run
            def dp(i, ph):
                def run():
                    def hval(p):
                        ld = lambda r: hb[zl, pl.ds(r, 8, stride=2), :]
                        if p < 0:
                            r = (p + P1) * SL
                            return (jnp.where(sub4 == 0, 0.0, ld(r - 1)), ld(r))
                        if p >= P1:
                            r = (p - P1) * SL
                            return (ld(r + 1), jnp.where(sub4 == 3, 0.0, ld(r + 2)))
                        return (ld(p * SL), ld(p * SL + 1))
                    d = [hval(2 * (8 * i + r) - 15 + ph) for r in range(15)]
                    for j, v in enumerate(_data_tree(d)):
                        d2[ph + zs, j, pl.ds(i * 8, 8), lanes(nt)] = _pk(*v)
                        yield
                return run
            return ([gel(s, b) for s in range(4) for b in range(B)],
                    [dp(i, ph) for i in range(5) for ph in range(2)])

        def post2_tasks(nt):
            def gel(s):
                def run():
                    ys = _out_tree([a2[nt % 2, 1 + zl, j, pl.ds(s * SL, SL), :] for j in range(NJ)])
                    for o, y in enumerate(ys):
                        y = _gelu(y)
                        fb[pl.ds((8 * s + o) * 8, 8), lanes(nt)] = _pk(y[:8], y[8:])
                        yield
                return run
            return [gel(s) for s in range(4)]

        for b in range(B):
            xb[0, :, pl.ds(4 * b * XP, 8), :] = jnp.zeros((NT, 8, 128), U32)
            xb[1, :, pl.ds((4 * b + 3) * XP + 60, 20), :] = jnp.zeros((NT, 20, 128), U32)
        for lt in range(NT):
            for b in range(B):
                for n in range(NCH):
                    xcopy(b, lt, n).start()
        dt = d1_tasks(0)
        for lt in range(NT):
            for b in range(B):
                for n in range(NCH):
                    xcopy(b, lt, n).wait()
            if lt == FL:
                for c in first:
                    c.start()
            _run(dt[lt * 8:(lt + 1) * 8])

        def unit(cv, nt, part, extra=(), ec=0, fine=False):
            _merge(dot_tasks(cv, nt, part, fine), 2 * NJ, (extra, ec))

        unit(0, 0, 0, d1_tasks(2), NJ, fine=True)
        wcopy(0, 1, 0).start()
        wcopy(0, 0, 1).wait()
        wcopy(0, 1, 1).start()
        unit(0, 0, 2, d1_tasks(1), NJ)
        unit(0, 0, 1)

        @pl.loop(1, NT)
        def _(nt):
            gl, dp = post1_tasks(nt - 1)
            ex = gl + dp
            for half in range(2):
                pl.when(nt < NT - 1)(lambda: wcopy(0, nt + 1, half).start())
                pl.when(nt == NT - 1)(lambda: wcopy(1, 1, half).start())
                wcopy(0, nt, half).wait()
            for half in range(2):
                unit(0, nt, 2 * half, ex[SP[half]:SP[half + 1]], NJ)
            pl.when(nt == 1)(lambda: wcopy(1, 0, 0).start())
            pl.when(nt == 2)(lambda: wcopy(1, 0, 1).start())
            unit(0, nt, 1, ex[SP[2]:], NJ)

        for grp in post1_tasks(NT - 1):
            _run(grp)
        def conv2(nt, start, extra):
            for c in range(2):
                for cc in (range(2) if c == 0 else ()) if MW else (c,):
                    start(cc)
                    wcopy(1, nt, cc).wait()
                unit(1, nt, c, extra[2 * c:2 * c + 2], 8)

        conv2(0, lambda c: wcopy(1, 2, c).start(), ())

        @pl.loop(1, NT)
        def _(nt):
            conv2(nt, lambda c: pl.when(nt == 1)(lambda: wcopy(1, 3, c).start()), post2_tasks(nt - 1))
            @pl.when(nt == 1)
            def _():
                for c in small:
                    c.start()

        _run(post2_tasks(NT - 1))
        for c in small:
            c.wait()
        feb[...] = jnp.dot(pltpu.bitcast(fb[...], BF16), wfb[...], preferred_element_type=F32)
        ge = jnp.dot(gb[...], wgb[...], preferred_element_type=F32)

        def out_copy(b, n, nrows):
            sl = pl.ds(n * P2 * U, nrows)
            return pltpu.make_async_copy(ob.at[b, sl, :], o_hbm.at[b, sl, :], sem_o.at[b * NCH + n])

        nts = [P2 if n < NCH - 1 else T2 - (NCH - 1) * P2 for n in range(NCH)]
        for b in range(B):
            geb = ge[b * U:(b + 1) * U]
            for n in range(NCH):
                rows = []
                for p in range(nts[n]):
                    r = feb[pl.ds(p * SL + 2 * n + b, 1), :]
                    rows.append(jnp.tanh(jnp.broadcast_to(r, (U, D)) + geb))
                j = jnp.concatenate(rows, axis=0).astype(BF16)
                o = jnp.dot(j, wob[...], preferred_element_type=F32)
                ob[b, pl.ds(n * P2 * U, nts[n] * U), :] = o.astype(BF16)
                out_copy(b, n, nts[n] * U).start()
        for b in range(B):
            for n in range(NCH):
                out_copy(b, n, nts[n] * U).wait()

    scratch = [
        pltpu.VMEM((2, NT, 8 * XP, 128), U32),
        pltpu.VMEM((2, NT, K, 256, 128), U32),
        [[pltpu.VMEM((2, 256, 128), F32)] * 18] * 2,
        pltpu.VMEM((B * U, D), BF16), pltpu.VMEM((D, D), BF16),
        pltpu.VMEM((D, D), BF16), pltpu.VMEM((D, D), BF16),
        pltpu.VMEM((3, 2, NJ, 32, D), U32), pltpu.VMEM((2, 3, NJ, 64, 128), F32),
        pltpu.VMEM((1, P1 * SL, 128), F32),
        pltpu.VMEM((2, NJ, 40, D), U32), pltpu.VMEM((2, 2, NJ, 64, 128), F32),
        pltpu.VMEM((P2 * 8, D), U32),
        pltpu.VMEM((P2 * SL, D), F32), pltpu.VMEM((B, T2 * U, D), BF16),
        pltpu.SemaphoreType.DMA((NT,)), pltpu.SemaphoreType.DMA((4 * NT,)),
        pltpu.SemaphoreType.DMA((4,)), pltpu.SemaphoreType.DMA((B * NCH,)),
        pltpu.SemaphoreType.REGULAR((2,)), pltpu.SemaphoreType.DMA((4,)),
    ]

    @jax.jit
    def fn(x, w1, w2, g, w_f, w_g, w_o):
        out = pl.pallas_call(
            kernel,
            out_shape=jax.ShapeDtypeStruct((B, T2 * U, D), x.dtype),
            in_specs=[pl.BlockSpec(memory_space=pl.ANY)] * 7,
            out_specs=pl.BlockSpec(memory_space=pl.ANY),
            scratch_shapes=scratch,
            compiler_params=pltpu.CompilerParams(vmem_limit_bytes=100 * 2**20),
        )(x, w1, w2, g.reshape(B * U, D), w_f, w_g, w_o)
        return out.reshape(B, T2, U, D)
    return fn


pallas_standalone__seq2seq_rnn_t_joint__speech_kernel = make()
```
